```python
import os as _os
_os.environ.setdefault("JAX_PLATFORMS", "cpu")
import jax
import jax.numpy as jnp

def _softmax(x, axis=-1):
    return jax.nn.softmax(x, axis=axis)
def _gelu(x):
    return jax.nn.gelu(x, approximate=True)
def _silu(x):
    return jax.nn.silu(x)
def _sigmoid(x):
    return jax.nn.sigmoid(x)
def _layernorm(x, axis=-1, eps=1e-5):
    m = jnp.mean(x, axis=axis, keepdims=True)
    v = jnp.var(x, axis=axis, keepdims=True)
    return (x - m) / jnp.sqrt(v + eps)
def _scatter_add(tgt, idx, src, axis=0):
    return tgt.at[idx].add(src)
def _segment_sum(src, seg, n):
    return jax.ops.segment_sum(src, seg, n)
class _Rng:
    def __init__(self, key):
        self._k = key
    def _next(self):
        self._k, sub = jax.random.split(self._k)
        return sub
    def normal(self, shape):
        return jax.random.normal(self._next(), shape, dtype=jnp.bfloat16)
    def randint(self, lo, hi, shape):
        return jax.random.randint(self._next(), shape, lo, hi, dtype=jnp.int32)
    def uniform(self, shape, lo=0.0, hi=1.0):
        return jax.random.uniform(self._next(), shape, jnp.bfloat16, lo, hi)
    def permutation(self, n):
        return jax.random.permutation(self._next(), n)


kernel_name = 'gated_mix__sliding_block_cached__dense_activation_silu__decode'

def setup_inputs():
    _rng = _Rng(jax.random.key(int.from_bytes(__import__("os").urandom(4), "little")))
    _w = (lambda a: (lambda t: t.astype(jnp.bfloat16) if jnp.issubdtype(t.dtype, jnp.floating) else t)(jnp.asarray(a)))
    def _A_setup():
        B, Sq, D = 2, 1, 1024
        Hq, Hkv, Sk, Dh = 32, 4, 32768, 128
        assert Hq % Hkv == 0, (Hq, Hkv)
        return {
            "x": _w((lambda *s: _rng.normal(s) * 0.05)(B, Sq, D)),
            "k_cache": _w((lambda *s: _rng.normal(s) * 3.2)(B, Hkv, Sk, Dh)),
            "v_cache": _w((lambda *s: _rng.normal(s) * 0.05)(B, Hkv, Sk, Dh)),
            "wq": _w((lambda *s: _rng.normal(s) * 3.2)(D, Hq * Dh) * (D ** -0.5)),
            "wo": _w((lambda *s: _rng.normal(s) * 0.05)(Hq * Dh, D) * ((Hq * Dh) ** -0.5)),
        }
    _A_in = _A_setup()

    def _B_setup():
        B, S, D, F = 2, 1, 1024, 3584
        return {
            "x": _w((lambda *s: _rng.normal(s) * 0.05)(B, S, D)),
            "w1": _w((lambda *s: _rng.normal(s) * 0.05)(D, F) * (D ** -0.5)),
            "w2": _w((lambda *s: _rng.normal(s) * 0.05)(F, D) * (F ** -0.5)),
        }
    _B_in = _B_setup()

    return {
        "A_x": _A_in["x"],
        "A_k_cache": _A_in["k_cache"],
        "A_v_cache": _A_in["v_cache"],
        "A_wq": _A_in["wq"],
        "A_wo": _A_in["wo"],
        "B_x": _B_in["x"],
        "B_w1": _B_in["w1"],
        "B_w2": _B_in["w2"],
        "gate_w": _w((lambda *s: _rng.normal(s) * 0.05)(1024) * 16.0),
    }

def reference(A_x, A_k_cache, A_v_cache, A_wq, A_wo, B_x, B_w1, B_w2, gate_w):
    def _A_ref(x, k_cache, v_cache, wq, wo):
        B, Sq, D = x.shape
        Hq, Dh = 32, 128
        Hkv, Sk = k_cache.shape[1], k_cache.shape[2]
        W = min(4096, max(256, Sk // 4))
        rep = Hq // Hkv
        q = (lambda x, *d: x.transpose(*d))((x @ wq).reshape(B, Sq, Hq, Dh), 0, 2, 1, 3)
        k = jnp.repeat(k_cache[:, :, Sk - W:, :], rep, axis=1)
        v = jnp.repeat(v_cache[:, :, Sk - W:, :], rep, axis=1)
        scores = jnp.einsum("bhqd,bhkd->bhqk", q, k) * (Dh ** -0.5)
        p = _softmax(scores, axis=-1)
        o = jnp.einsum("bhqk,bhkd->bhqd", p, v)
        return (lambda x, *d: x.transpose(*d))(o, 0, 2, 1, 3).reshape(B, Sq, Hq * Dh) @ wo

    def _B_ref(x, w1, w2):
        h = jnp.einsum("bsd,df->bsf", x, w1)
        h = _silu(h)
        out = jnp.einsum("bsf,fd->bsd", h, w2)
        return out

    x = A_x
    g = _sigmoid((x * gate_w).sum(-1, keepdims=True))
    a = _A_ref(x, A_k_cache, A_v_cache, A_wq, A_wo)
    b = _B_ref(x, B_w1, B_w2)
    return g * a + (1 - g) * b
```

```python
import jax
import jax.numpy as jnp
from jax import lax
import jax.experimental.pallas as pl
import jax.experimental.pallas.tpu as pltpu

_BF = jnp.bfloat16
_F32 = jnp.float32


def _build(B, D, Hkv, Sk, Dh, HD, F, *, fc=512, ahead=2, prio=True, nobc=True):
    rep = HD // (Dh * Hkv)
    G = rep * Dh
    W = min(4096, max(256, Sk // 4))
    NF = F // fc
    NB = B * Hkv
    scale = Dh ** -0.5
    R = B * rep
    assert F % fc == 0 and rep == 8 and B == 2

    def kernel(x_hbm, k_hbm, v_hbm, wq_hbm, wo_hbm, w1_hbm, w2_hbm, gw_hbm, o_hbm,
               xb, gb, ob, wqb, kb, vb, wob, w1b, w2b, qs, ps, ls, os_, hs, sem, sem_s):
        def c_wq(i):
            return wq_hbm.at[:, pl.ds(pl.multiple_of(i * G, G), G)], wqb.at[i]
        def c_k(i):
            return k_hbm.at[i % B, i // B, pl.ds(Sk - W, W), :], kb.at[i]
        def c_v(i):
            return v_hbm.at[i % B, i // B, pl.ds(Sk - W, W), :], vb.at[i]
        def c_wo(i):
            return wo_hbm.at[pl.ds(pl.multiple_of(i * G, G), G), :], wob.at[i]
        def c_w1(i):
            return w1_hbm.at[:, pl.ds(pl.multiple_of(i * fc, fc), fc)], w1b.at[i]
        def c_w2(i):
            return w2_hbm.at[pl.ds(pl.multiple_of(i * fc, fc), fc), :], w2b.at[i]
        phases = [(c_wq, Hkv), (c_k, NB), (c_v, NB), (c_wo, Hkv), (c_w1, NF), (c_w2, NF)]

        def cp(ph, i):
            s, d = phases[ph][0](i)
            return pltpu.make_async_copy(s, d, sem.at[ph, i])

        def start(ph, i):
            if not prio:
                cp(ph, i).start()
            elif isinstance(i, int):
                cp(ph, i).start(priority=i % 2)
            else:
                @pl.when(i % 2 == 0)
                def _():
                    cp(ph, i).start(priority=0)
                @pl.when(i % 2 == 1)
                def _():
                    cp(ph, i).start(priority=1)

        def run(ph, body, init=None):
            n = phases[ph][1]

            def step(i, c):
                cp(ph, i).wait()
                @pl.when(i + ahead < n)
                def _():
                    start(ph, jnp.minimum(i + ahead, n - 1))
                if ph + 1 < len(phases):
                    @pl.when(i + ahead >= n)
                    def _():
                        start(ph + 1, jnp.maximum(i + ahead - n, 0))
                return body(i, c)
            return lax.fori_loop(0, n, step, init)

        for i in range(ahead):
            start(0, i)
        cx = pltpu.make_async_copy(x_hbm, xb, sem_s.at[0])
        cg = pltpu.make_async_copy(gw_hbm, gb, sem_s.at[1])
        cx.start()
        cg.start()
        cx.wait()
        cg.wait()

        row = lax.broadcasted_iota(jnp.int32, (R, Dh), 0) % rep
        xf = [xb[b].astype(_F32) for b in range(B)]
        x16 = jnp.concatenate([jnp.broadcast_to(v, (rep, D)) for v in xf], 0).astype(_BF)

        def q_body(g, _):
            r = jnp.dot(x16, wqb[g], preferred_element_type=_F32)
            q = r[:, :Dh]
            for j in range(1, rep):
                q = jnp.where(row == j, r[:, j * Dh:(j + 1) * Dh], q)
            qs[g] = q
        run(0, q_body)

        def rows(i):
            return pl.ds(pl.multiple_of((i % B) * rep, rep), rep)

        def k_body(i, _):
            q = qs[i // B, rows(i), :].astype(_BF)
            s = lax.dot_general(q, kb[i], (((1,), (1,)), ((), ())),
                                preferred_element_type=_F32) * scale
            p = jnp.exp(s - jnp.max(s, axis=-1, keepdims=True))
            ps[i] = p
            ls[i] = jnp.broadcast_to(1.0 / jnp.sum(p, axis=-1, keepdims=True), (rep, Dh))
        run(1, k_body)

        def v_body(i, _):
            o = jnp.dot(ps[i].astype(_BF), vb[i], preferred_element_type=_F32)
            os_[i // B, rows(i), :] = o * ls[i]
        run(2, v_body)

        def o_body(g, acc):
            o = os_[g]
            lhs = jnp.concatenate([jnp.where(row == j, o, 0.0) for j in range(rep)], 1)
            return acc + jnp.dot(lhs.astype(_BF), wob[g], preferred_element_type=_F32)
        acc = run(3, o_body, jnp.zeros((R, D), _F32))

        gw = gb[...].astype(_F32).reshape(1, D)
        r8 = lax.broadcasted_iota(jnp.int32, (8, D), 0)
        x8 = jnp.where(r8 == 0, xf[0], xf[1])
        gate = jax.nn.sigmoid(jnp.sum(x8 * gw, axis=-1, keepdims=True))
        a8 = jnp.where(r8 == 0, jnp.sum(acc[:rep], 0, keepdims=True),
                       jnp.sum(acc[rep:], 0, keepdims=True))
        ga = gate * a8
        x8b = x8.astype(_BF)

        def h_body(i, _):
            h = jnp.dot(x8b, w1b[i], preferred_element_type=_F32)
            hs[i] = h * jax.nn.sigmoid(h)
        run(4, h_body)

        def f_body(i, acc):
            return acc + jnp.dot(hs[i].astype(_BF), w2b[i], preferred_element_type=_F32)
        ff = run(5, f_body, jnp.zeros((8, D), _F32))

        res = ga + (1.0 - gate) * ff
        for b in range(B):
            ob[b] = res[b:b + 1].astype(_BF)
        co = pltpu.make_async_copy(ob, o_hbm, sem_s.at[0])
        co.start()
        co.wait()

    hbm = pl.BlockSpec(memory_space=pl.ANY)
    return pl.pallas_call(
        kernel,
        out_shape=jax.ShapeDtypeStruct((B, 1, D), _BF),
        in_specs=[hbm] * 8,
        out_specs=hbm,
        scratch_shapes=[
            pltpu.VMEM((B, 1, D), _BF), pltpu.VMEM((D,), _BF), pltpu.VMEM((B, 1, D), _BF),
            pltpu.VMEM((Hkv, D, G), _BF), pltpu.VMEM((NB, W, Dh), _BF),
            pltpu.VMEM((NB, W, Dh), _BF), pltpu.VMEM((Hkv, G, D), _BF),
            pltpu.VMEM((NF, D, fc), _BF), pltpu.VMEM((NF, fc, D), _BF),
            pltpu.VMEM((Hkv, R, Dh), _F32), pltpu.VMEM((NB, rep, W), _F32),
            pltpu.VMEM((NB, rep, Dh), _F32), pltpu.VMEM((Hkv, R, Dh), _F32),
            pltpu.VMEM((NF, 8, fc), _F32),
            pltpu.SemaphoreType.DMA((6, max(NB, NF))), pltpu.SemaphoreType.DMA((2,)),
        ],
        compiler_params=pltpu.CompilerParams(vmem_limit_bytes=100 << 20,
                                             disable_bounds_checks=nobc),
    )


@jax.jit
def pallas_gated_mix__sliding_block_cached__dense_activation_silu__decode_kernel(
    A_x, A_k_cache, A_v_cache, A_wq, A_wo, B_x, B_w1, B_w2, gate_w,
):
    B, _, D = A_x.shape
    _, Hkv, Sk, Dh = A_k_cache.shape
    call = _build(B, D, Hkv, Sk, Dh, A_wq.shape[1], B_w1.shape[1])
    return call(A_x, A_k_cache, A_v_cache, A_wq, A_wo, B_w1, B_w2, gate_w)
```

```python
import jax
import jax.numpy as jnp
from jax import lax
import jax.experimental.pallas as pl
import jax.experimental.pallas.tpu as pltpu

_BF = jnp.bfloat16
_F32 = jnp.float32


def _build(B, D, Hkv, Sk, Dh, HD, F, *, fc=512, ahead=4, prio=True, nobc=True, fl=256, nl=4):
    rep = HD // (Dh * Hkv)
    G = rep * Dh
    W = min(4096, max(256, Sk // 4))
    NF = F // fc
    NB = B * Hkv
    F2 = F - fl * nl
    N2 = F2 // fc
    assert F2 % fc == 0 and N2 >= 1
    scale = Dh ** -0.5
    R = B * rep
    assert F % fc == 0 and rep == 8 and B == 2

    def kernel(x_hbm, k_hbm, v_hbm, wq_hbm, wo_hbm, w1_hbm, w2_hbm, gw_hbm, o_hbm,
               xb, gb, ob, wqb, kb, vb, wob, w1b, w2b, w2l, qs, ps, ls, os_, hs, sem, sem_s):
        def c_wq(i):
            return wq_hbm.at[:, pl.ds(pl.multiple_of(i * G, G), G)], wqb.at[i]
        def c_k(i):
            return k_hbm.at[i % B, i // B, pl.ds(Sk - W, W), :], kb.at[i]
        def c_v(i):
            return v_hbm.at[i % B, i // B, pl.ds(Sk - W, W), :], vb.at[i]
        def c_wo(i):
            return wo_hbm.at[pl.ds(pl.multiple_of(i * G, G), G), :], wob.at[i]
        def c_w1(i):
            return w1_hbm.at[:, pl.ds(pl.multiple_of(i * fc, fc), fc)], w1b.at[i]
        def c_w2(i):
            return w2_hbm.at[pl.ds(pl.multiple_of(i * fc, fc), fc), :], w2b.at[i]
        def c_w2l(i):
            return w2_hbm.at[pl.ds(pl.multiple_of(F2 + i * fl, fl), fl), :], w2l.at[i]
        phases = [(c_wq, Hkv), (c_k, NB), (c_v, NB), (c_wo, Hkv), (c_w1, NF), (c_w2, N2),
                  (c_w2l, nl)]

        def cp(ph, i):
            s, d = phases[ph][0](i)
            return pltpu.make_async_copy(s, d, sem.at[ph, i])

        def start(ph, i):
            o = sum(n for _, n in phases[:ph])
            if not prio:
                cp(ph, i).start()
            elif isinstance(i, int):
                cp(ph, i).start(priority=(i + o) % 2)
            else:
                @pl.when((i + o) % 2 == 0)
                def _():
                    cp(ph, i).start(priority=0)
                @pl.when((i + o) % 2 == 1)
                def _():
                    cp(ph, i).start(priority=1)

        def run(ph, body, init=None):
            n = phases[ph][1]

            def step(i, c):
                cp(ph, i).wait()
                lo = 0
                for p2 in range(ph, len(phases)):
                    m = phases[p2][1]
                    if lo < n + ahead and lo + m > ahead:
                        t = i + ahead - lo
                        pl.when((t >= 0) & (t < m))(
                            lambda p2=p2, t=t, m=m: start(p2, jnp.clip(t, 0, m - 1)))
                    lo += m
                return body(i, c)
            return lax.fori_loop(0, n, step, init)

        cx = pltpu.make_async_copy(x_hbm, xb, sem_s.at[0])
        cg = pltpu.make_async_copy(gw_hbm, gb, sem_s.at[1])
        start(0, 0)
        cx.start(priority=1)
        cg.start(priority=1)
        flat = [(ph, i) for ph, (_, n) in enumerate(phases) for i in range(n)]
        for ph, i in flat[1:ahead]:
            start(ph, i)
        cx.wait()
        cg.wait()

        row = lax.broadcasted_iota(jnp.int32, (R, Dh), 0) % rep
        xv = xb[...].astype(_F32)
        xf = [xv[b:b + 1] for b in range(B)]
        x16 = jnp.concatenate([jnp.broadcast_to(v, (rep, D)) for v in xf], 0).astype(_BF)

        def q_body(g, _):
            r = jnp.dot(x16, wqb[g], preferred_element_type=_F32)
            q = r[:, :Dh]
            for j in range(1, rep):
                q = jnp.where(row == j, r[:, j * Dh:(j + 1) * Dh], q)
            qs[g] = q
        run(0, q_body)

        def rows(i):
            return pl.ds(pl.multiple_of((i % B) * rep, rep), rep)

        def k_body(i, _):
            q = qs[i // B, rows(i), :].astype(_BF)
            s = lax.dot_general(q, kb[i], (((1,), (1,)), ((), ())),
                                preferred_element_type=_F32) * scale
            p = jnp.exp(s - jnp.max(s, axis=-1, keepdims=True))
            ps[i] = p
            ls[i] = jnp.broadcast_to(1.0 / jnp.sum(p, axis=-1, keepdims=True), (rep, Dh))
        run(1, k_body)

        def v_body(i, _):
            o = jnp.dot(ps[i].astype(_BF), vb[i], preferred_element_type=_F32)
            os_[i // B, rows(i), :] = o * ls[i]
        run(2, v_body)

        def o_body(g, acc):
            o = os_[g]
            lhs = jnp.concatenate([jnp.where(row == j, o, 0.0) for j in range(rep)], 1)
            return acc + jnp.dot(lhs.astype(_BF), wob[g], preferred_element_type=_F32)
        acc = run(3, o_body, jnp.zeros((R, D), _F32))

        gw = gb[...].astype(_F32).reshape(1, D)
        r8 = lax.broadcasted_iota(jnp.int32, (8, D), 0)
        x8 = jnp.where(r8 == 0, xf[0], xf[1])
        gate = jax.nn.sigmoid(jnp.sum(x8 * gw, axis=-1, keepdims=True))
        a8 = jnp.where(r8 == 0, jnp.sum(acc[:rep], 0, keepdims=True),
                       jnp.sum(acc[rep:], 0, keepdims=True))
        ga = gate * a8
        x8b = x8.astype(_BF)

        def h_body(i, _):
            h = jnp.dot(x8b, w1b[i], preferred_element_type=_F32)
            hs[:, pl.ds(pl.multiple_of(i * fc, fc), fc)] = h * jax.nn.sigmoid(h)
        run(4, h_body)

        def f_body(i, acc):
            return acc + jnp.dot(hs[:, pl.ds(pl.multiple_of(i * fc, fc), fc)].astype(_BF), w2b[i], preferred_element_type=_F32)
        ff = run(5, f_body, jnp.zeros((8, D), _F32))

        def l_body(i, acc):
            h = hs[:, pl.ds(pl.multiple_of(F2 + i * fl, fl), fl)].astype(_BF)
            return acc + jnp.dot(h, w2l[i], preferred_element_type=_F32)
        ff = run(6, l_body, ff)

        res = ga + (1.0 - gate) * ff
        ob[...] = res[:B].astype(_BF)
        co = pltpu.make_async_copy(ob, o_hbm, sem_s.at[0])
        co.start()
        co.wait()

    hbm = pl.BlockSpec(memory_space=pl.ANY)
    return pl.pallas_call(
        kernel,
        out_shape=jax.ShapeDtypeStruct((B, D), _BF),
        in_specs=[hbm] * 8,
        out_specs=hbm,
        scratch_shapes=[
            pltpu.VMEM((B, D), _BF), pltpu.VMEM((D,), _BF), pltpu.VMEM((B, D), _BF),
            pltpu.VMEM((Hkv, D, G), _BF), pltpu.VMEM((NB, W, Dh), _BF),
            pltpu.VMEM((NB, W, Dh), _BF), pltpu.VMEM((Hkv, G, D), _BF),
            pltpu.VMEM((NF, D, fc), _BF), pltpu.VMEM((N2, fc, D), _BF),
            pltpu.VMEM((nl, fl, D), _BF),
            pltpu.VMEM((Hkv, R, Dh), _F32), pltpu.VMEM((NB, rep, W), _F32),
            pltpu.VMEM((NB, rep, Dh), _F32), pltpu.VMEM((Hkv, R, Dh), _F32),
            pltpu.VMEM((8, F), _F32),
            pltpu.SemaphoreType.DMA((7, max(NB, NF, nl))), pltpu.SemaphoreType.DMA((2,)),
        ],
        compiler_params=pltpu.CompilerParams(vmem_limit_bytes=100 << 20,
                                             disable_bounds_checks=nobc),
    )


def _wrap(A_x, A_k_cache, A_v_cache, A_wq, A_wo, B_x, B_w1, B_w2, gate_w, **kw):
    B, _, D = A_x.shape
    _, Hkv, Sk, Dh = A_k_cache.shape
    call = _build(B, D, Hkv, Sk, Dh, A_wq.shape[1], B_w1.shape[1], **kw)
    out = call(A_x.reshape(B, D), A_k_cache, A_v_cache, A_wq, A_wo, B_w1, B_w2, gate_w)
    return out.reshape(B, 1, D)


@jax.jit
def pallas_gated_mix__sliding_block_cached__dense_activation_silu__decode_kernel(
    A_x, A_k_cache, A_v_cache, A_wq, A_wo, B_x, B_w1, B_w2, gate_w,
):
    return _wrap(A_x, A_k_cache, A_v_cache, A_wq, A_wo, B_x, B_w1, B_w2, gate_w)
```
